```python
import os as _os
_os.environ.setdefault("JAX_PLATFORMS", "cpu")
import jax
import jax.numpy as jnp

def _softmax(x, axis=-1):
    return jax.nn.softmax(x, axis=axis)
def _gelu(x):
    return jax.nn.gelu(x, approximate=True)
def _silu(x):
    return jax.nn.silu(x)
def _sigmoid(x):
    return jax.nn.sigmoid(x)
def _layernorm(x, axis=-1, eps=1e-5):
    m = jnp.mean(x, axis=axis, keepdims=True)
    v = jnp.var(x, axis=axis, keepdims=True)
    return (x - m) / jnp.sqrt(v + eps)
def _scatter_add(tgt, idx, src, axis=0):
    return tgt.at[idx].add(src)
def _segment_sum(src, seg, n):
    return jax.ops.segment_sum(src, seg, n)
class _Rng:
    def __init__(self, key):
        self._k = key
    def _next(self):
        self._k, sub = jax.random.split(self._k)
        return sub
    def normal(self, shape):
        return jax.random.normal(self._next(), shape, dtype=jnp.bfloat16)
    def randint(self, lo, hi, shape):
        return jax.random.randint(self._next(), shape, lo, hi, dtype=jnp.int32)
    def uniform(self, shape, lo=0.0, hi=1.0):
        return jax.random.uniform(self._next(), shape, jnp.bfloat16, lo, hi)
    def permutation(self, n):
        return jax.random.permutation(self._next(), n)


kernel_name = 'standalone__linear_kernel_hedgehog__prompt'

def setup_inputs():
    _rng = _Rng(jax.random.key(int.from_bytes(__import__("os").urandom(4), "little")))
    _w = (lambda a: (lambda t: t.astype(jnp.bfloat16) if jnp.issubdtype(t.dtype, jnp.floating) else t)(jnp.asarray(a)))
    B, S, D, H = 1, 2048, 1024, 32
    Dh = D // H
    return {
        "x": _w((lambda *s: _rng.normal(s) * 0.4)(B, S, D)),
        "wqkv": _w((lambda *s: _rng.normal(s) * 0.4)(D, 3 * D)),
        "w_phi": _w((lambda *s: _rng.normal(s) * 0.4)(H, Dh, Dh) * (Dh ** -0.5)),
        "wo": _w((lambda *s: _rng.normal(s) * 0.05)(D, D)),
    }

def reference(x, wqkv, w_phi, wo):
    B, S, D = x.shape
    H = 32; Dh = D // H
    qkv = (lambda x, *d: x.transpose(*d))((x @ wqkv).reshape(B, S, 3, H, Dh), 2, 0, 3, 1, 4)
    q, k, v = qkv[0], qkv[1], qkv[2]
    pq = jnp.einsum("bhsd,hdf->bhsf", q, w_phi)
    pk = jnp.einsum("bhsd,hdf->bhsf", k, w_phi)
    phi_q = jnp.concatenate([_softmax(pq, axis=-1), _softmax(-pq, axis=-1)], axis=-1)
    phi_k = jnp.concatenate([_softmax(pk, axis=-1), _softmax(-pk, axis=-1)], axis=-1)
    kv = jnp.einsum("bhsf,bhsd->bhfd", phi_k, v)
    z  = jnp.einsum("bhsf->bhf", phi_k)
    num = jnp.einsum("bhqf,bhfd->bhqd", phi_q, kv)
    den = jnp.einsum("bhqf,bhf->bhq", phi_q, z)[..., None] + 1e-6
    o = num / den
    return (lambda x, *d: x.transpose(*d))(o, 0, 2, 1, 3).reshape(B, S, D) @ wo
```

```python
import functools

import jax
import jax.numpy as jnp
from jax import lax
import jax.experimental.pallas as pl
import jax.experimental.pallas.tpu as pltpu

H = 32
DH = 32
HPG = 4
GW = HPG * DH
TM = 512
LHS_ROWS = 144

_NT = (((1,), (1,)), ((), ()))
_TT = (((0,), (1,)), ((), ()))


def _dual_softmax(p):
    tm = p.shape[-1]
    p3 = p.reshape(HPG, DH, tm)
    mx = jnp.max(p3, axis=1, keepdims=True)
    mn = jnp.min(p3, axis=1, keepdims=True)
    e1 = jnp.exp(p3 - mx)
    e2 = jnp.exp(mn - p3)
    r1 = 1.0 / jnp.sum(e1, axis=1, keepdims=True)
    r2 = 1.0 / jnp.sum(e2, axis=1, keepdims=True)
    return (e1 * r1).reshape(GW, tm), (e2 * r2).reshape(GW, tm)


def _kernel(x_ref, wqkv_ref, wphi_ref, wo_ref, o_ref,
            wfold, phiq, kv_acc, z_acc, lhs, *, D, G):
    phase = pl.program_id(0)
    i = pl.program_id(1)
    bf16 = jnp.bfloat16
    f32 = jnp.float32

    @pl.when(jnp.logical_and(phase == 0, i == 0))
    def _init():
        row = lax.broadcasted_iota(jnp.int32, (GW, GW), 0) // DH
        col = lax.broadcasted_iota(jnp.int32, (GW, GW), 1) // DH
        bd = row == col
        for g in range(G):
            w = wphi_ref[g * GW:(g + 1) * GW, :]
            wt = jnp.concatenate([w] * HPG, axis=1)
            wbd = jnp.where(bd, wt, jnp.zeros_like(wt))
            for part in range(2):
                c0 = part * D + g * GW
                wcols = wqkv_ref[:, c0:c0 + GW]
                res = lax.dot_general(wbd, wcols, _TT, preferred_element_type=f32)
                wfold[c0:c0 + GW, :] = res.astype(bf16)
        kv_acc[...] = jnp.zeros_like(kv_acc)
        z_acc[...] = jnp.zeros_like(z_acc)

    @pl.when(phase == 0)
    def _phase0():
        x = x_ref[...]
        v = jnp.dot(x, wqkv_ref[:, 2 * D:3 * D], preferred_element_type=f32).astype(bf16)
        pT = lax.dot_general(wfold[...], x, _NT, preferred_element_type=f32)
        for g in range(G):
            qp, qn = _dual_softmax(pT[g * GW:(g + 1) * GW])
            phiq[i, 2 * g * GW:(2 * g + 1) * GW, :] = qp.astype(bf16)
            phiq[i, (2 * g + 1) * GW:(2 * g + 2) * GW, :] = qn.astype(bf16)
            kp, kn = _dual_softmax(pT[D + g * GW:D + (g + 1) * GW])
            phik = jnp.concatenate([kp, kn], axis=0)
            zp = phik[:, 0:128]
            for t in range(1, TM // 128):
                zp = zp + phik[:, t * 128:(t + 1) * 128]
            z_acc[g] += zp
            kv_acc[g] += jnp.dot(phik.astype(bf16), v[:, g * GW:(g + 1) * GW],
                                 preferred_element_type=f32)

    @pl.when(phase == 1)
    def _phase1():
        @pl.when(i == 0)
        def _prep():
            r = lax.broadcasted_iota(jnp.int32, (GW, 2 * GW), 0) // DH
            c = (lax.broadcasted_iota(jnp.int32, (GW, 2 * GW), 1) % GW) // DH
            m_kv = r == c
            r2 = lax.broadcasted_iota(jnp.int32, (LHS_ROWS - GW, 2 * GW), 0)
            c2 = (lax.broadcasted_iota(jnp.int32, (LHS_ROWS - GW, 2 * GW), 1) % GW) // DH
            m_z = r2 == c2
            for g in range(G):
                kvT = kv_acc[g].T
                lhs[g, 0:GW, :] = jnp.where(m_kv, kvT, 0.0).astype(bf16)
                zrow = jnp.sum(z_acc[g].T, axis=0, keepdims=True)
                zb = jnp.broadcast_to(zrow, (LHS_ROWS - GW, 2 * GW))
                lhs[g, GW:LHS_ROWS, :] = jnp.where(m_z, zb, 0.0).astype(bf16)

        oTs = []
        for g in range(G):
            r = jnp.dot(lhs[g], phiq[i, 2 * g * GW:(2 * g + 2) * GW, :],
                        preferred_element_type=f32)
            num = r[0:GW].reshape(HPG, DH, TM)
            den = r[GW:GW + 8]
            rec = 1.0 / (den + 1e-6)
            rec = rec[0:HPG].reshape(HPG, 1, TM)
            oTs.append((num * rec).reshape(GW, TM))
        oT = jnp.concatenate(oTs, axis=0)
        o = oT.T.astype(bf16)
        o_ref[...] = jnp.dot(o, wo_ref[...], preferred_element_type=f32).astype(o_ref.dtype)


@jax.jit
def pallas_standalone__linear_kernel_hedgehog__prompt_kernel(
    x: jax.Array,
    wqkv: jax.Array,
    w_phi: jax.Array,
    wo: jax.Array,
):
    B, S, D = x.shape
    assert B == 1 and D == H * DH and S % TM == 0
    G = D // GW
    nt = S // TM
    x2 = x.reshape(S, D)
    wphi2 = w_phi.reshape(H * DH, DH)

    out = pl.pallas_call(
        functools.partial(_kernel, D=D, G=G),
        grid=(2, nt),
        in_specs=[
            pl.BlockSpec((TM, D), lambda p, i: (i * (1 - p) + (nt - 1) * p, 0)),
            pl.BlockSpec((D, 3 * D), lambda p, i: (0, 0)),
            pl.BlockSpec((H * DH, DH), lambda p, i: (0, 0)),
            pl.BlockSpec((D, D), lambda p, i: (0, 0)),
        ],
        out_specs=pl.BlockSpec((TM, D), lambda p, i: (i * p, 0)),
        out_shape=jax.ShapeDtypeStruct((S, D), x.dtype),
        scratch_shapes=[
            pltpu.VMEM((2 * D, D), jnp.bfloat16),
            pltpu.VMEM((nt, 2 * D, TM), jnp.bfloat16),
            pltpu.VMEM((G, 2 * GW, GW), jnp.float32),
            pltpu.VMEM((G, 2 * GW, 128), jnp.float32),
            pltpu.VMEM((G, LHS_ROWS, 2 * GW), jnp.bfloat16),
        ],
        compiler_params=pltpu.CompilerParams(
            dimension_semantics=("arbitrary", "arbitrary"),
            vmem_limit_bytes=100 * 1024 * 1024,
        ),
    )(x2, wqkv, wphi2, wo)
    return out.reshape(B, S, D)
```

```python
import functools

import jax
import jax.numpy as jnp
from jax import lax
import jax.experimental.pallas as pl
import jax.experimental.pallas.tpu as pltpu

H = 32
DH = 32
HPG = 4
GW = HPG * DH
TM = 512
NVC = 2
NOC = 4
PW = 2 * DH
PR = PW + 16

_NT = (((1,), (1,)), ((), ()))
_TT = (((0,), (1,)), ((), ()))


def _dual_softmax(p):
    tm = p.shape[-1]
    p3 = p.reshape(2, DH, tm)
    mx = jnp.max(p3, axis=1, keepdims=True)
    mn = jnp.min(p3, axis=1, keepdims=True)
    e1 = jnp.exp(p3 - mx)
    e2 = jnp.exp(mn - p3)
    r1 = 1.0 / jnp.sum(e1, axis=1, keepdims=True)
    r2 = 1.0 / jnp.sum(e2, axis=1, keepdims=True)
    return jnp.concatenate([(e1 * r1).reshape(PW, tm), (e2 * r2).reshape(PW, tm)], axis=0)


def _kernel(x_hbm, wqkv_hbm, wphi_hbm, wo_hbm, o_hbm,
            x_v, w_v, wphi_ref, wo_v, out_v, v0_v, vt_v, wfold, kv_acc, lhs,
            x_sem, x0_sem, wv_sem, w_sem, o_sem, *, D, G, NT):
    bf16 = jnp.bfloat16
    f32 = jnp.float32
    HM = TM // 2
    VC = D // NVC
    OC = D // NOC
    NP = D // PW

    def x_copy(t):
        return pltpu.make_async_copy(x_hbm.at[pl.ds(t * TM, TM), :], x_v.at[t], x_sem.at[t])

    def x0_copy(h):
        return pltpu.make_async_copy(x_hbm.at[pl.ds(h * HM, HM), :],
                                     x_v.at[0, pl.ds(h * HM, HM), :], x0_sem.at[h])

    def wv_copy(c):
        return pltpu.make_async_copy(wqkv_hbm.at[:, pl.ds(2 * D + c * VC, VC)],
                                     w_v.at[2, :, pl.ds(c * VC, VC)], wv_sem.at[c])

    def w_copy(part):
        return pltpu.make_async_copy(wqkv_hbm.at[:, pl.ds(part * D, D)],
                                     w_v.at[part], w_sem.at[part])

    def wphi_copy():
        return pltpu.make_async_copy(wphi_hbm, wphi_ref, w_sem.at[2])

    def wo_copy():
        return pltpu.make_async_copy(wo_hbm, wo_v, w_sem.at[3])

    def o_copy(t, c):
        return pltpu.make_async_copy(out_v.at[t, :, pl.ds(c * OC, OC)],
                                     o_hbm.at[pl.ds(t * TM, TM), pl.ds(c * OC, OC)],
                                     o_sem.at[t * NOC + c])

    def fold(part):
        row = lax.broadcasted_iota(jnp.int32, (GW, GW), 0) // DH
        col = lax.broadcasted_iota(jnp.int32, (GW, GW), 1) // DH
        bd = row == col
        for g in range(G):
            w = wphi_ref[g * GW:(g + 1) * GW, :]
            wt = jnp.concatenate([w] * HPG, axis=1)
            wbd = jnp.where(bd, wt, jnp.zeros_like(wt))
            wcols = w_v[part, :, g * GW:(g + 1) * GW]
            res = lax.dot_general(wbd, wcols, _TT, preferred_element_type=f32)
            wfold[part, g * GW:(g + 1) * GW, :] = res.astype(bf16)

    def k_tile(x, v):
        vt = v.T.astype(bf16)
        for j in range(NP):
            vt_v[j, 0:PW, :] = vt[j * PW:(j + 1) * PW]
        pT = lax.dot_general(wfold[1], x, _NT, preferred_element_type=f32)
        for j in range(NP):
            phik = _dual_softmax(pT[j * PW:(j + 1) * PW]).astype(bf16)
            kv_acc[j] += lax.dot_general(vt_v[j], phik, _NT, preferred_element_type=f32)

    def prep():
        r = lax.broadcasted_iota(jnp.int32, (PR, 2 * PW), 0)
        c = (lax.broadcasted_iota(jnp.int32, (PR, 2 * PW), 1) % PW) // DH
        rh = jnp.where(r < PW, r // DH, r - PW)
        m = rh == c
        for j in range(NP):
            lhs[j] = jnp.where(m, kv_acc[j], 0.0).astype(bf16)

    def q_tile(t):
        x = x_v[t]
        pT = lax.dot_general(wfold[0], x, _NT, preferred_element_type=f32)
        oTs = []
        for j in range(NP):
            phiq = _dual_softmax(pT[j * PW:(j + 1) * PW]).astype(bf16)
            r = jnp.dot(lhs[j], phiq, preferred_element_type=f32)
            num = r[0:PW].reshape(2, DH, TM)
            den = r[PW:PW + 8]
            rec = 1.0 / (den + 1e-6)
            rec = rec[0:2].reshape(2, 1, TM)
            oTs.append((num * rec).reshape(PW, TM))
        oT = jnp.concatenate(oTs, axis=0)
        o = oT.T.astype(bf16)
        for c in range(NOC):
            out_v[t, :, c * OC:(c + 1) * OC] = jnp.dot(
                o, wo_v[:, c * OC:(c + 1) * OC], preferred_element_type=f32).astype(bf16)
            o_copy(t, c).start()

    x0_copy(0).start()
    wv_copy(0).start()
    x0_copy(1).start()
    for c in range(1, NVC):
        wv_copy(c).start()
    wphi_copy().start()
    w_copy(1).start()
    for t in range(1, NT):
        x_copy(t).start()
    w_copy(0).start()
    wo_copy().start()
    kv_acc[...] = jnp.zeros_like(kv_acc)
    vt_v[:, PW:PR, :] = jnp.ones((NP, PR - PW, TM), bf16)

    x0_copy(0).wait()
    wv_copy(0).wait()
    v0_v[0:HM, 0:VC] = jnp.dot(x_v[0, 0:HM, :], w_v[2, :, 0:VC],
                               preferred_element_type=f32)
    x0_copy(1).wait()
    v0_v[HM:TM, 0:VC] = jnp.dot(x_v[0, HM:TM, :], w_v[2, :, 0:VC],
                                preferred_element_type=f32)
    for c in range(1, NVC):
        wv_copy(c).wait()
        v0_v[:, c * VC:(c + 1) * VC] = jnp.dot(x_v[0], w_v[2, :, c * VC:(c + 1) * VC],
                                               preferred_element_type=f32)
    wphi_copy().wait()
    w_copy(1).wait()
    fold(1)
    k_tile(x_v[0], v0_v[...])
    w_copy(0).wait()
    fold(0)

    def body0(t, carry):
        x_copy(t).wait()
        x = x_v[t]
        v = jnp.dot(x, w_v[2], preferred_element_type=f32)
        k_tile(x, v)
        return carry
    lax.fori_loop(1, NT, body0, 0)

    wo_copy().wait()
    prep()
    q_tile(0)

    def body1(t, carry):
        q_tile(t)
        return carry
    lax.fori_loop(1, NT, body1, 0)

    for t in range(NT):
        for c in range(NOC):
            o_copy(t, c).wait()


@jax.jit
def pallas_standalone__linear_kernel_hedgehog__prompt_kernel(
    x: jax.Array,
    wqkv: jax.Array,
    w_phi: jax.Array,
    wo: jax.Array,
):
    B, S, D = x.shape
    assert B == 1 and D == H * DH and S % TM == 0
    G = D // GW
    nt = S // TM
    x2 = x.reshape(S, D)
    wphi2 = w_phi.reshape(H * DH, DH)

    out = pl.pallas_call(
        functools.partial(_kernel, D=D, G=G, NT=nt),
        in_specs=[
            pl.BlockSpec(memory_space=pl.ANY),
            pl.BlockSpec(memory_space=pl.ANY),
            pl.BlockSpec(memory_space=pl.ANY),
            pl.BlockSpec(memory_space=pl.ANY),
        ],
        out_specs=pl.BlockSpec(memory_space=pl.ANY),
        out_shape=jax.ShapeDtypeStruct((S, D), x.dtype),
        scratch_shapes=[
            pltpu.VMEM((nt, TM, D), jnp.bfloat16),
            pltpu.VMEM((3, D, D), jnp.bfloat16),
            pltpu.VMEM((H * DH, DH), jnp.bfloat16),
            pltpu.VMEM((D, D), jnp.bfloat16),
            pltpu.VMEM((nt, TM, D), jnp.bfloat16),
            pltpu.VMEM((TM, D), jnp.float32),
            pltpu.VMEM((D // PW, PR, TM), jnp.bfloat16),
            pltpu.VMEM((2, D, D), jnp.bfloat16),
            pltpu.VMEM((D // PW, PR, 2 * PW), jnp.float32),
            pltpu.VMEM((D // PW, PR, 2 * PW), jnp.bfloat16),
            pltpu.SemaphoreType.DMA((nt,)),
            pltpu.SemaphoreType.DMA((2,)),
            pltpu.SemaphoreType.DMA((NVC,)),
            pltpu.SemaphoreType.DMA((4,)),
            pltpu.SemaphoreType.DMA((nt * NOC,)),
        ],
        compiler_params=pltpu.CompilerParams(
            vmem_limit_bytes=100 * 1024 * 1024,
        ),
    )(x2, wqkv, wphi2, wo)
    return out.reshape(B, S, D)
```

```python
import functools

import jax
import jax.numpy as jnp
from jax import lax
import jax.experimental.pallas as pl
import jax.experimental.pallas.tpu as pltpu

H = 32
DH = 32
HPG = 4
GW = HPG * DH
TM = 512
NVC = 2
OCH = ((0, 512), (512, 256), (768, 128), (896, 128))
NOC = len(OCH)
PW = 2 * DH
PF = 2 * PW

_NT = (((1,), (1,)), ((), ()))
_TT = (((0,), (1,)), ((), ()))


def _dual_softmax(p):
    tm = p.shape[-1]
    p3 = p.reshape(2, DH, tm)
    mx = jnp.max(p3, axis=1, keepdims=True)
    mn = jnp.min(p3, axis=1, keepdims=True)
    e1 = jnp.exp(p3 - mx)
    e2 = jnp.exp(mn - p3)
    r1 = 1.0 / jnp.sum(e1, axis=1, keepdims=True)
    r2 = 1.0 / jnp.sum(e2, axis=1, keepdims=True)
    return jnp.concatenate([(e1 * r1).reshape(PW, tm), (e2 * r2).reshape(PW, tm)], axis=0)


def _kernel(x_hbm, wqkv_hbm, wphi_hbm, wo_hbm, o_hbm,
            x_v, w_v, wphi_ref, wo_v, out_v, v0_v, wfold, kv_acc, z_acc, lhs, zb,
            x_sem, x0_sem, wv_sem, w_sem, o_sem, *, D, G, NT):
    bf16 = jnp.bfloat16
    f32 = jnp.float32
    HM = TM // 2
    VC = D // NVC
    NP = D // PW

    def x_copy(t):
        return pltpu.make_async_copy(x_hbm.at[pl.ds(t * TM, TM), :], x_v.at[t], x_sem.at[t])

    def x0_copy(h):
        return pltpu.make_async_copy(x_hbm.at[pl.ds(h * HM, HM), :],
                                     x_v.at[0, pl.ds(h * HM, HM), :], x0_sem.at[h])

    def wv_copy(c):
        return pltpu.make_async_copy(wqkv_hbm.at[:, pl.ds(2 * D + c * VC, VC)],
                                     w_v.at[2, :, pl.ds(c * VC, VC)], wv_sem.at[c])

    def w_copy(part):
        return pltpu.make_async_copy(wqkv_hbm.at[:, pl.ds(part * D, D)],
                                     w_v.at[part], w_sem.at[part])

    def wphi_copy():
        return pltpu.make_async_copy(wphi_hbm, wphi_ref, w_sem.at[2])

    def wo_copy():
        return pltpu.make_async_copy(wo_hbm, wo_v, w_sem.at[3])

    def o_copy(t, c):
        c0, cw = OCH[c]
        return pltpu.make_async_copy(out_v.at[t, :, pl.ds(c0, cw)],
                                     o_hbm.at[pl.ds(t * TM, TM), pl.ds(c0, cw)],
                                     o_sem.at[t * NOC + c])

    def fold(part):
        row = lax.broadcasted_iota(jnp.int32, (GW, GW), 0) // DH
        col = lax.broadcasted_iota(jnp.int32, (GW, GW), 1) // DH
        bd = row == col
        for g in range(G):
            w = wphi_ref[g * GW:(g + 1) * GW, :]
            wt = jnp.concatenate([w] * HPG, axis=1)
            wbd = jnp.where(bd, wt, jnp.zeros_like(wt))
            wcols = w_v[part, :, g * GW:(g + 1) * GW]
            res = lax.dot_general(wbd, wcols, _TT, preferred_element_type=f32)
            wfold[part, g * GW:(g + 1) * GW, :] = res.astype(bf16)

    def k_tile(x, v):
        pT = lax.dot_general(wfold[1], x, _NT, preferred_element_type=f32)
        if v is None:
            v = jnp.dot(x, w_v[2], preferred_element_type=f32)
        vt = v.T.astype(bf16)
        for j in range(NP):
            phik = _dual_softmax(pT[j * PW:(j + 1) * PW])
            zp = phik[:, 0:128]
            for l in range(1, TM // 128):
                zp = zp + phik[:, l * 128:(l + 1) * 128]
            z_acc[j] += zp
            kv_acc[j] += lax.dot_general(vt[j * PW:(j + 1) * PW], phik.astype(bf16), _NT,
                                         preferred_element_type=f32)

    def prep():
        r = lax.broadcasted_iota(jnp.int32, (PW, PF), 0) // DH
        c = (lax.broadcasted_iota(jnp.int32, (PW, PF), 1) % PW) // DH
        m = r == c
        for j in range(NP):
            lhs[j] = jnp.where(m, kv_acc[j], 0.0).astype(bf16)
            z = jnp.sum(z_acc[j], axis=1, keepdims=True)
            zb[j] = jnp.broadcast_to(z, (PF, 128))

    def q_tile(t):
        x = x_v[t]
        pT = lax.dot_general(wfold[0], x, _NT, preferred_element_type=f32)
        oTs = []
        for j in range(NP):
            phiq = _dual_softmax(pT[j * PW:(j + 1) * PW])
            num = jnp.dot(lhs[j], phiq.astype(bf16), preferred_element_type=f32)
            zj = zb[j]
            wz = phiq * jnp.concatenate([zj] * (TM // 128), axis=1)
            den = jnp.sum(wz.reshape(2, 2, DH, TM), axis=2)
            den = den[0] + den[1]
            rec = 1.0 / (den + 1e-6)
            oTs.append((num.reshape(2, DH, TM) * rec.reshape(2, 1, TM)).reshape(PW, TM))
        oT = jnp.concatenate(oTs, axis=0)
        o = oT.T.astype(bf16)
        for c in range(NOC):
            c0, cw = OCH[c]
            out_v[t, :, c0:c0 + cw] = jnp.dot(
                o, wo_v[:, c0:c0 + cw], preferred_element_type=f32).astype(bf16)
            o_copy(t, c).start()

    x0_copy(0).start()
    wv_copy(0).start()
    x0_copy(1).start()
    for c in range(1, NVC):
        wv_copy(c).start()
    wphi_copy().start()
    w_copy(1).start()
    for t in range(1, NT):
        x_copy(t).start()
    w_copy(0).start()
    wo_copy().start()
    kv_acc[...] = jnp.zeros_like(kv_acc)
    z_acc[...] = jnp.zeros_like(z_acc)

    x0_copy(0).wait()
    wv_copy(0).wait()
    v0_v[0:HM, 0:VC] = jnp.dot(x_v[0, 0:HM, :], w_v[2, :, 0:VC],
                               preferred_element_type=f32)
    x0_copy(1).wait()
    v0_v[HM:TM, 0:VC] = jnp.dot(x_v[0, HM:TM, :], w_v[2, :, 0:VC],
                                preferred_element_type=f32)
    for c in range(1, NVC):
        wv_copy(c).wait()
        v0_v[:, c * VC:(c + 1) * VC] = jnp.dot(x_v[0], w_v[2, :, c * VC:(c + 1) * VC],
                                               preferred_element_type=f32)
    wphi_copy().wait()
    w_copy(1).wait()
    fold(1)
    k_tile(x_v[0], v0_v[...])
    w_copy(0).wait()
    fold(0)

    def body0(t, carry):
        x_copy(t).wait()
        k_tile(x_v[t], None)
        return carry
    lax.fori_loop(1, NT, body0, 0)

    wo_copy().wait()
    prep()
    q_tile(0)

    def body1(t, carry):
        q_tile(t)
        return carry
    lax.fori_loop(1, NT, body1, 0)

    for t in range(NT):
        for c in range(NOC):
            o_copy(t, c).wait()


@jax.jit
def pallas_standalone__linear_kernel_hedgehog__prompt_kernel(
    x: jax.Array,
    wqkv: jax.Array,
    w_phi: jax.Array,
    wo: jax.Array,
):
    B, S, D = x.shape
    assert B == 1 and D == H * DH and S % TM == 0
    assert OCH[-1][0] + OCH[-1][1] == D
    G = D // GW
    nt = S // TM
    x2 = x.reshape(S, D)
    wphi2 = w_phi.reshape(H * DH, DH)

    out = pl.pallas_call(
        functools.partial(_kernel, D=D, G=G, NT=nt),
        in_specs=[
            pl.BlockSpec(memory_space=pl.ANY),
            pl.BlockSpec(memory_space=pl.ANY),
            pl.BlockSpec(memory_space=pl.ANY),
            pl.BlockSpec(memory_space=pl.ANY),
        ],
        out_specs=pl.BlockSpec(memory_space=pl.ANY),
        out_shape=jax.ShapeDtypeStruct((S, D), x.dtype),
        scratch_shapes=[
            pltpu.VMEM((nt, TM, D), jnp.bfloat16),
            pltpu.VMEM((3, D, D), jnp.bfloat16),
            pltpu.VMEM((H * DH, DH), jnp.bfloat16),
            pltpu.VMEM((D, D), jnp.bfloat16),
            pltpu.VMEM((nt, TM, D), jnp.bfloat16),
            pltpu.VMEM((TM, D), jnp.float32),
            pltpu.VMEM((2, D, D), jnp.bfloat16),
            pltpu.VMEM((D // PW, PW, PF), jnp.float32),
            pltpu.VMEM((D // PW, PF, 128), jnp.float32),
            pltpu.VMEM((D // PW, PW, PF), jnp.bfloat16),
            pltpu.VMEM((D // PW, PF, 128), jnp.float32),
            pltpu.SemaphoreType.DMA((nt,)),
            pltpu.SemaphoreType.DMA((2,)),
            pltpu.SemaphoreType.DMA((NVC,)),
            pltpu.SemaphoreType.DMA((4,)),
            pltpu.SemaphoreType.DMA((nt * NOC,)),
        ],
        compiler_params=pltpu.CompilerParams(
            vmem_limit_bytes=100 * 1024 * 1024,
        ),
    )(x2, wqkv, wphi2, wo)
    return out.reshape(B, S, D)
```
